```python
import os as _os
_os.environ.setdefault("JAX_PLATFORMS", "cpu")
import jax
import jax.numpy as jnp

def _softmax(x, axis=-1):
    return jax.nn.softmax(x, axis=axis)
def _gelu(x):
    return jax.nn.gelu(x, approximate=True)
def _silu(x):
    return jax.nn.silu(x)
def _sigmoid(x):
    return jax.nn.sigmoid(x)
def _layernorm(x, axis=-1, eps=1e-5):
    m = jnp.mean(x, axis=axis, keepdims=True)
    v = jnp.var(x, axis=axis, keepdims=True)
    return (x - m) / jnp.sqrt(v + eps)
def _scatter_add(tgt, idx, src, axis=0):
    return tgt.at[idx].add(src)
def _segment_sum(src, seg, n):
    return jax.ops.segment_sum(src, seg, n)
class _Rng:
    def __init__(self, key):
        self._k = key
    def _next(self):
        self._k, sub = jax.random.split(self._k)
        return sub
    def normal(self, shape):
        return jax.random.normal(self._next(), shape, dtype=jnp.bfloat16)
    def randint(self, lo, hi, shape):
        return jax.random.randint(self._next(), shape, lo, hi, dtype=jnp.int32)
    def uniform(self, shape, lo=0.0, hi=1.0):
        return jax.random.uniform(self._next(), shape, jnp.bfloat16, lo, hi)
    def permutation(self, n):
        return jax.random.permutation(self._next(), n)


kernel_name = 'sequential_preLN__spectral_gfnet__glu_gated_bilinear__prompt'

def setup_inputs():
    _rng = _Rng(jax.random.key(int.from_bytes(__import__("os").urandom(4), "little")))
    _w = (lambda a: (lambda t: t.astype(jnp.bfloat16) if jnp.issubdtype(t.dtype, jnp.floating) else t)(jnp.asarray(a)))
    def _A_setup():
        B, S, D = 1, 2048, 448
        Df = D // 2 + 1
        return {
            "x": _w((lambda *s: _rng.normal(s) * 0.05)(B, S, D)),
            "w_r": _w((lambda *s: _rng.normal(s) * 0.2)(S, Df) * 0.02),
            "w_i": _w((lambda *s: _rng.normal(s) * 0.2)(S, Df) * 0.02),
        }
    _A_in = _A_setup()

    def _B_setup():
        B, S, D, F = 1, 2048, 448, 1792
        return {
            "x": _w((lambda *s: _rng.normal(s) * 0.05)(B, S, D)),
            "w_gate": _w((lambda *s: _rng.normal(s) * 0.05)(D, F) * (D ** -0.5)),
            "w_up": _w((lambda *s: _rng.normal(s) * 0.05)(D, F) * (D ** -0.5)),
            "w_down": _w((lambda *s: _rng.normal(s) * 0.05)(F, D) * (F ** -0.5)),
        }
    _B_in = _B_setup()

    return {
        "A_x": _A_in["x"],
        "A_w_r": _A_in["w_r"],
        "A_w_i": _A_in["w_i"],
        "B_x": _B_in["x"],
        "B_w_gate": _B_in["w_gate"],
        "B_w_up": _B_in["w_up"],
        "B_w_down": _B_in["w_down"],
    }

def reference(A_x, A_w_r, A_w_i, B_x, B_w_gate, B_w_up, B_w_down):
    def _A_ref(x, w_r, w_i):
        B, S, D = x.shape
        X = (lambda x, axes=(-2,-1): jnp.fft.rfft2(x.astype(jnp.float32), axes=axes))(x, axes=(-2, -1))
        W = w_r + 1j * w_i
        X = X * W
        y = (lambda x, s, axes=(-2,-1): jnp.fft.irfft2(x, s=s, axes=axes).astype(jnp.bfloat16))(X, (S, D), axes=(-2, -1))
        return y

    def _B_ref(x, w_gate, w_up, w_down):
        g = jnp.einsum("bsd,df->bsf", x, w_gate)
        u = jnp.einsum("bsd,df->bsf", x, w_up)
        h = g * u
        return jnp.einsum("bsf,fd->bsd", h, w_down)

    x = A_x
    h = x + _A_ref(_layernorm(x, axis=-1), A_w_r, A_w_i)
    h2 = h + _B_ref(_layernorm(h, axis=-1), B_w_gate, B_w_up, B_w_down)
    return h2
```

```python
import functools

import numpy as np
import jax
import jax.numpy as jnp
import jax.experimental.pallas as pl
import jax.experimental.pallas.tpu as pltpu

S = 2048
D = 448
DF = D // 2 + 1
RP = 240
R2 = 2 * RP
F = 1792
N1 = 16
N2 = S // N1
TN = 512
NCH = S // TN
EPS = 1e-5


@functools.lru_cache(maxsize=None)
def _tables():
    d = np.arange(D)[None, :]
    k = np.arange(DF)[:, None]
    ang = 2.0 * np.pi * ((d * k) % D) / D
    fwd = np.zeros((R2, D), np.float64)
    fwd[:DF, :] = np.cos(ang)
    fwd[RP:RP + DF, :] = -np.sin(ang)
    c = np.full((DF,), 2.0)
    c[0] = 1.0
    c[DF - 1] = 1.0
    inv = np.zeros((D, R2), np.float64)
    inv[:, :DF] = (c[None, :] * np.cos(ang.T)) / (S * D)
    inv[:, RP:RP + DF] = -(c[None, :] * np.sin(ang.T)) / (S * D)
    n = np.arange(N2)
    ang2 = 2.0 * np.pi * ((n[:, None] * n[None, :]) % N2) / N2
    cs = np.concatenate([np.cos(ang2), np.sin(ang2)], axis=1)
    k1 = np.arange(N1)[:, None]
    ang3 = (2.0 * np.pi * ((k1 * n[None, :]) % S) / S).reshape(1, S)
    twc = np.broadcast_to(np.cos(ang3), (8, S))
    tws = np.broadcast_to(np.sin(ang3), (8, S))
    return (fwd.astype(np.float32), inv.astype(np.float32), cs.astype(np.float32),
            np.ascontiguousarray(twc, np.float32), np.ascontiguousarray(tws, np.float32))


def _cfft(xs, sign):
    n = len(xs)
    if n == 1:
        return xs
    ev = _cfft(xs[0::2], sign)
    od = _cfft(xs[1::2], sign)
    out = [None] * n
    for q in range(n // 2):
        er, ei = ev[q]
        orr, oi = od[q]
        if q == 0:
            tr, ti = orr, oi
        elif 4 * q == n:
            if sign < 0:
                tr, ti = oi, -orr
            else:
                tr, ti = -oi, orr
        else:
            a = 2.0 * np.pi * q / n
            wc, ws = float(np.cos(a)), float(sign * np.sin(a))
            tr = orr * wc - oi * ws
            ti = orr * ws + oi * wc
        out[q] = (er + tr, ei + ti)
        out[q + n // 2] = (er - tr, ei - ti)
    return out


def _ln_t(xf):
    m = jnp.mean(xf, axis=0, keepdims=True)
    xc = xf - m
    v = jnp.mean(xc * xc, axis=0, keepdims=True)
    return xc * jax.lax.rsqrt(v + EPS)


def _kernel(x_ref, wr_hbm, wi_hbm, wg_hbm, wu_hbm, wd_hbm,
            fwd_ref, inv_ref, cs_ref, twc_ref, tws_ref,
            o_ref, z_ref, wgt_ref, wut_ref, wrn_ref, win_ref,
            wr_ref, wi_ref, wg_ref, wu_ref, wd_ref, sems):
    step = pl.program_id(0)

    def _copies():
        pairs = ((wr_hbm, wr_ref), (wi_hbm, wi_ref), (wg_hbm, wg_ref),
                 (wu_hbm, wu_ref), (wd_hbm, wd_ref))
        return [pltpu.make_async_copy(src, dst, sems.at[n])
                for n, (src, dst) in enumerate(pairs)]

    @pl.when(step == 0)
    def _spectral():
        cps = _copies()
        for cp in cps:
            cp.start()
        def p1(i, carry):
            cl = pl.ds(pl.multiple_of(i * TN, TN), TN)
            z = _ln_t(x_ref[:, cl].astype(jnp.float32)).astype(jnp.bfloat16)
            z_ref[:, cl] = jnp.dot(fwd_ref[...], z, preferred_element_type=jnp.float32)
            return carry
        jax.lax.fori_loop(0, NCH, p1, 0)

        cps[0].wait()
        cps[1].wait()
        for src, dst in ((wr_ref, wrn_ref), (wi_ref, win_ref)):
            wn = src[...].astype(jnp.float32).T
            dst[0] = wn[:, :128]
            dst[1] = jnp.zeros((S, 128), jnp.float32)
            dst[1, :, :DF - 128] = wn[:, 128:]

        RB = 8

        def p2(j, carry):
            rr = pl.ds(pl.multiple_of(j * RB, RB), RB)
            ri = pl.ds(pl.multiple_of(RP + j * RB, RB), RB)
            xs = []
            for b in range(N1):
                cl = slice(b * N2, (b + 1) * N2)
                xs.append((z_ref[rr, cl], z_ref[ri, cl]))
            ys = _cfft(xs, -1)
            for b in range(N1):
                cl = slice(b * N2, (b + 1) * N2)
                yr, yi = ys[b]
                if b > 0:
                    c = twc_ref[:, cl]
                    s = tws_ref[:, cl]
                    yr, yi = yr * c + yi * s, yi * c - yr * s
                z_ref[rr, cl] = yr
                z_ref[ri, cl] = yi
            return carry
        jax.lax.fori_loop(0, RP // RB, p2, 0)

        for b in range(N1):
            cl = slice(b * N2, (b + 1) * N2)
            a = z_ref[:, cl].astype(jnp.bfloat16)
            p = jnp.dot(a, cs_ref[...], preferred_element_type=jnp.float32)
            xr = p[:RP, :N2] + p[RP:, N2:]
            xi = p[RP:, :N2] - p[:RP, N2:]
            sl = pl.ds(b, N2, stride=N1)
            wr = jnp.concatenate([wrn_ref[0, sl, :], wrn_ref[1, sl, :]], axis=1).T[:RP]
            wi = jnp.concatenate([win_ref[0, sl, :], win_ref[1, sl, :]], axis=1).T[:RP]
            yr = xr * wr - xi * wi
            yi = xr * wi + xi * wr
            y = jnp.concatenate([yr, yi], axis=0).astype(jnp.bfloat16)
            q = jnp.dot(y, cs_ref[...], preferred_element_type=jnp.float32)
            z_ref[:RP, cl] = q[:RP, :N2] - q[RP:, N2:]
            z_ref[RP:, cl] = q[RP:, :N2] + q[:RP, N2:]

        def p4(j, carry):
            rr = pl.ds(pl.multiple_of(j * RB, RB), RB)
            ri = pl.ds(pl.multiple_of(RP + j * RB, RB), RB)
            xs = []
            for b in range(N1):
                cl = slice(b * N2, (b + 1) * N2)
                yr, yi = z_ref[rr, cl], z_ref[ri, cl]
                if b > 0:
                    c = twc_ref[:, cl]
                    s = tws_ref[:, cl]
                    yr, yi = yr * c - yi * s, yi * c + yr * s
                xs.append((yr, yi))
            ys = _cfft(xs, +1)
            for b in range(N1):
                cl = slice(b * N2, (b + 1) * N2)
                z_ref[rr, cl] = ys[b][0]
                z_ref[ri, cl] = ys[b][1]
            return carry
        jax.lax.fori_loop(0, RP // RB, p4, 0)

        cps[2].wait()
        wgt_ref[...] = wg_ref[...].T
        cps[3].wait()
        wut_ref[...] = wu_ref[...].T
        cps[4].wait()

    @pl.when(step > 0)
    def _ffn():
        i = step - 1
        cl = pl.ds(pl.multiple_of(i * TN, TN), TN)
        y = jnp.dot(inv_ref[...], z_ref[:, cl].astype(jnp.bfloat16),
                    preferred_element_type=jnp.float32)
        h = x_ref[:, cl].astype(jnp.float32) + y.astype(jnp.bfloat16).astype(jnp.float32)
        h = h.astype(jnp.bfloat16).astype(jnp.float32)
        l2 = _ln_t(h).astype(jnp.bfloat16)
        g = jnp.dot(wgt_ref[...], l2, preferred_element_type=jnp.float32)
        u = jnp.dot(wut_ref[...], l2, preferred_element_type=jnp.float32)
        hh = (g * u).astype(jnp.bfloat16)
        o = jnp.dot(wd_ref[...], hh, preferred_element_type=jnp.float32)
        o_ref[...] = (h + o).astype(o_ref.dtype)


@jax.jit
def pallas_sequential_preLN__spectral_gfnet__glu_gated_bilinear__prompt_kernel(
    A_x: jax.Array,
    A_w_r: jax.Array,
    A_w_i: jax.Array,
    B_x: jax.Array,
    B_w_gate: jax.Array,
    B_w_up: jax.Array,
    B_w_down: jax.Array,
):
    fwd, inv, cs, twc, tws = _tables()
    xt = A_x.reshape(S, D).T

    perm = lambda w: w.T

    wdt = B_w_down.T
    hbm = pl.BlockSpec(memory_space=pl.ANY)
    full = lambda shape: pl.BlockSpec(shape, lambda i: (0,) * len(shape))
    out = pl.pallas_call(
        _kernel,
        grid=(NCH + 1,),
        in_specs=[
            full((D, S)), hbm, hbm, hbm, hbm, hbm,
            full((R2, D)), full((D, R2)), full((N2, 2 * N2)),
            full((8, S)), full((8, S)),
        ],
        out_specs=pl.BlockSpec((D, TN), lambda i: (0, jnp.maximum(i - 1, 0))),
        out_shape=jax.ShapeDtypeStruct((D, S), jnp.bfloat16),
        scratch_shapes=[
            pltpu.VMEM((R2, S), jnp.float32),
            pltpu.VMEM((F, D), jnp.bfloat16),
            pltpu.VMEM((F, D), jnp.bfloat16),
            pltpu.VMEM((2, S, 128), jnp.float32),
            pltpu.VMEM((2, S, 128), jnp.float32),
            pltpu.VMEM((DF, S), jnp.bfloat16),
            pltpu.VMEM((DF, S), jnp.bfloat16),
            pltpu.VMEM((D, F), jnp.bfloat16),
            pltpu.VMEM((D, F), jnp.bfloat16),
            pltpu.VMEM((D, F), jnp.bfloat16),
            pltpu.SemaphoreType.DMA((5,)),
        ],
        compiler_params=pltpu.CompilerParams(
            dimension_semantics=("arbitrary",),
            vmem_limit_bytes=100 * 1024 * 1024,
        ),
    )(xt, perm(A_w_r), perm(A_w_i), B_w_gate, B_w_up, wdt,
      jnp.asarray(fwd, jnp.bfloat16), jnp.asarray(inv, jnp.bfloat16),
      jnp.asarray(cs, jnp.bfloat16), jnp.asarray(twc), jnp.asarray(tws))
    return out.T.reshape(1, S, D)
```
